```python
import os as _os
_os.environ.setdefault("JAX_PLATFORMS", "cpu")
import jax
import jax.numpy as jnp

def _softmax(x, axis=-1):
    return jax.nn.softmax(x, axis=axis)
def _gelu(x):
    return jax.nn.gelu(x, approximate=True)
def _silu(x):
    return jax.nn.silu(x)
def _sigmoid(x):
    return jax.nn.sigmoid(x)
def _layernorm(x, axis=-1, eps=1e-5):
    m = jnp.mean(x, axis=axis, keepdims=True)
    v = jnp.var(x, axis=axis, keepdims=True)
    return (x - m) / jnp.sqrt(v + eps)
def _scatter_add(tgt, idx, src, axis=0):
    return tgt.at[idx].add(src)
def _segment_sum(src, seg, n):
    return jax.ops.segment_sum(src, seg, n)
class _Rng:
    def __init__(self, key):
        self._k = key
    def _next(self):
        self._k, sub = jax.random.split(self._k)
        return sub
    def normal(self, shape):
        return jax.random.normal(self._next(), shape, dtype=jnp.bfloat16)
    def randint(self, lo, hi, shape):
        return jax.random.randint(self._next(), shape, lo, hi, dtype=jnp.int32)
    def uniform(self, shape, lo=0.0, hi=1.0):
        return jax.random.uniform(self._next(), shape, jnp.bfloat16, lo, hi)
    def permutation(self, n):
        return jax.random.permutation(self._next(), n)


kernel_name = 'interleave_layers__linear_kernel_hedgehog__sliding_block__prompt'

def setup_inputs():
    _rng = _Rng(jax.random.key(int.from_bytes(__import__("os").urandom(4), "little")))
    _w = (lambda a: (lambda t: t.astype(jnp.bfloat16) if jnp.issubdtype(t.dtype, jnp.floating) else t)(jnp.asarray(a)))
    def _A_setup():
        B, S, D, H = 1, 2048, 448, 16
        Dh = D // H
        return {
            "x": _w((lambda *s: _rng.normal(s) * 0.05)(B, S, D)),
            "wqkv": _w((lambda *s: _rng.normal(s) * 0.4)(D, 3 * D)),
            "w_phi": _w((lambda *s: _rng.normal(s) * 0.4)(H, Dh, Dh) * (Dh ** -0.5)),
            "wo": _w((lambda *s: _rng.normal(s) * 0.05)(D, D)),
        }
    _A_in = _A_setup()

    def _B_setup():
        B, S, D = 1, 2048, 448
        return {
            "x": _w((lambda *s: _rng.normal(s) * 0.05)(B, S, D)),
            "wqkv": _w((lambda *s: _rng.normal(s) * 0.1)(D, 3 * D)),
            "wo": _w((lambda *s: _rng.normal(s) * 0.1)(D, D)),
        }
    _B_in = _B_setup()

    return {
        "A_x": _A_in["x"],
        "A_wqkv": _A_in["wqkv"],
        "A_w_phi": _A_in["w_phi"],
        "A_wo": _A_in["wo"],
        "B_x": _B_in["x"],
        "B_wqkv": _B_in["wqkv"],
        "B_wo": _B_in["wo"],
    }

def reference(A_x, A_wqkv, A_w_phi, A_wo, B_x, B_wqkv, B_wo):
    def _A_ref(x, wqkv, w_phi, wo):
        B, S, D = x.shape
        H = 16; Dh = D // H
        qkv = (lambda x, *d: x.transpose(*d))((x @ wqkv).reshape(B, S, 3, H, Dh), 2, 0, 3, 1, 4)
        q, k, v = qkv[0], qkv[1], qkv[2]
        pq = jnp.einsum("bhsd,hdf->bhsf", q, w_phi)
        pk = jnp.einsum("bhsd,hdf->bhsf", k, w_phi)
        phi_q = jnp.concatenate([_softmax(pq, axis=-1), _softmax(-pq, axis=-1)], axis=-1)
        phi_k = jnp.concatenate([_softmax(pk, axis=-1), _softmax(-pk, axis=-1)], axis=-1)
        kv = jnp.einsum("bhsf,bhsd->bhfd", phi_k, v)
        z  = jnp.einsum("bhsf->bhf", phi_k)
        num = jnp.einsum("bhqf,bhfd->bhqd", phi_q, kv)
        den = jnp.einsum("bhqf,bhf->bhq", phi_q, z)[..., None] + 1e-6
        o = num / den
        return (lambda x, *d: x.transpose(*d))(o, 0, 2, 1, 3).reshape(B, S, D) @ wo

    def _B_ref(x, wqkv, wo):
        B, S, D = x.shape
        H = 16; Dh = D // H; W = 256
        qkv = (lambda x, *d: x.transpose(*d))((x @ wqkv).reshape(B, S, 3, H, Dh), 2, 0, 3, 1, 4)
        q, k, v = qkv[0], qkv[1], qkv[2]
        scores = jnp.einsum("bhqd,bhkd->bhqk", q, k) * (Dh ** -0.5)
        idx = jnp.arange(S)
        mask = (idx[:, None] - idx[None, :] >= 0) & (idx[:, None] - idx[None, :] < W)
        scores = jnp.where(mask[None, None], scores, -1e9)
        p = _softmax(scores, axis=-1)
        o = jnp.einsum("bhqk,bhkd->bhqd", p, v)
        return (lambda x, *d: x.transpose(*d))(o, 0, 2, 1, 3).reshape(B, S, D) @ wo

    x = A_x
    x = x + _A_ref(_layernorm(x, axis=-1), A_wqkv, A_w_phi, A_wo)
    x = x + _B_ref(_layernorm(x, axis=-1), B_wqkv, B_wo)
    x = x + _A_ref(_layernorm(x, axis=-1), A_wqkv, A_w_phi, A_wo)
    x = x + _B_ref(_layernorm(x, axis=-1), B_wqkv, B_wo)
    return x
```

```python
import jax
import jax.numpy as jnp
from jax import lax
import jax.experimental.pallas as pl
import jax.experimental.pallas.tpu as pltpu

S, D, H, DH = 2048, 448, 16, 28
NP = H // 2
PR = 2 * DH
T = 128
LOG2E = 1.4426950408889634
F32, BF16, I32 = jnp.float32, jnp.bfloat16, jnp.int32
C = 512
NC = S // C
Q = dict(f0=400, f1=200, m0=200, m1=100, m2=50, m3=600, m4=0.9, m5=300, m6=1500, ns0=4, lag0=5,
         w0=1, w1=1200, w2=5000, w3=1.0, wl=0.98, bs=1, ns1=3, lag1=3, t0=5000, t1=200, ns3=4, lag3=3)
DM = (0, 0, 2, 2, 0, 4) + (4,) * 7
QS = (1, 3, 5, 6)
INREG, YS = (), 4
NS, MUTOK, RS, PVF = 3, False, 112, False
G, LAG = 1, 3
LEV = dict(aqkv=1, ao=1, bqkv=1, bo=1)
FLAGS = {}


def _iota(shape, axis):
    return lax.broadcasted_iota(I32, shape, axis)


def _dot(a, b):
    return jnp.dot(a, b, preferred_element_type=F32)


def _dot_nt(a, b):
    return lax.dot_general(a, b, (((1,), (1,)), ((), ())), preferred_element_type=F32)


def _tree(op, xs):
    xs = list(xs)
    while len(xs) > 1:
        xs = [op(xs[i], xs[i + 1]) if i + 1 < len(xs) else xs[i] for i in range(0, len(xs), 2)]
    return xs[0]


def _chains(op, xs, n=2):
    accs = list(xs[:n])
    for i, v in enumerate(xs[n:]):
        accs[i % n] = op(accs[i % n], v)
    return _tree(op, accs)


def _i32(x):
    return pltpu.bitcast(x, I32)


def _bf16(x):
    return pltpu.bitcast(x, BF16)


def _pack(x):
    return jnp.concatenate([_i32(pltpu.pack_elementwise([x[r:r + 8], x[r + 8:r + 16]], packed_dtype=BF16))
                            for r in range(0, x.shape[0], 16)], axis=0)


def _unpack(w):
    return jnp.concatenate([pltpu.unpack_elementwise(w, index=i, packed_dtype=BF16, unpacked_dtype=F32)
                            for i in (0, 1)], axis=0)


def _rows8(x):
    return [x[r:r + 8] for r in range(0, x.shape[0], 8)]


def _allreduce8(op, v, shifts):
    for s in shifts:
        v = op(v, pltpu.roll(v, s, 0))
    return v


def _hedgehog(p):
    rows = _rows8(p)
    hi = _allreduce8(jnp.maximum, _tree(jnp.maximum, rows), (4, 2))
    lo = _allreduce8(jnp.minimum, _tree(jnp.minimum, rows), (4, 2))
    out = []
    for e in ([jnp.exp2(r - hi) for r in rows], [jnp.exp2(lo - r) for r in rows]):
        inv = _recip(_allreduce8(jnp.add, _tree(jnp.add, e), (4, 2)))
        out += [v * inv for v in e]
    return _pack(jnp.concatenate(out, axis=0))


def _add(u, v):
    return [x + y for x, y in zip(u, v)]


def _sub(u, v):
    return [x - y for x, y in zip(u, v)]


def _recip(x):
    r = pl.reciprocal(x, approx=True)
    return r * (2.0 - x * r)


def _split_lhs(ks):
    if len(ks) == 1:
        return [ks[0]]
    m, h = ks[0].shape[0] // 2, len(ks) // 2
    a11, a12 = [k[:m] for k in ks[:h]], [k[:m] for k in ks[h:]]
    a21, a22 = [k[m:] for k in ks[:h]], [k[m:] for k in ks[h:]]
    ops = [_add(a21, a22), a22, a11, _add(a11, a12), _add(a11, a22), _sub(a21, a11), _sub(a12, a22)]
    return [p for o in ops for p in _split_lhs(o)]


def _split_rhs(ks):
    if len(ks) == 1:
        return [_pack(ks[0])]
    n, h = ks[0].shape[1] // 2, len(ks) // 2
    b11, b12 = [k[:, :n] for k in ks[:h]], [k[:, n:] for k in ks[:h]]
    b21, b22 = [k[:, :n] for k in ks[h:]], [k[:, n:] for k in ks[h:]]
    ops = [b11, _sub(b21, b11), _sub(b12, b22), b22, _add(b11, b22), _add(b11, b12), _add(b21, b22)]
    return [p for o in ops for p in _split_rhs(o)]


class _Buf:
    def __init__(self, ref, cols):
        self.ref, self.cols = ref, cols

    def at(self, i):
        return _Buf(self.ref.at[i], self.cols)

    def panels(self, idx):
        idx = idx if isinstance(idx, tuple) else (idx,)
        idx += (slice(None),) * (len(self.ref.shape) - 1 - len(idx))
        lo, hi, _ = idx[-1].indices(self.cols)
        return [idx[:-2] + (l // T, idx[-2], slice(0, min(T, hi - l))) for l in range(lo, hi, T)]

    def __setitem__(self, idx, v):
        for i, at in enumerate(self.panels(idx)):
            part = v[:, i * T:(i + 1) * T]
            if self.ref.dtype == BF16:
                self.ref[at] = part.astype(BF16)
            else:
                if part.shape[1] < T:
                    part = jnp.concatenate([part, jnp.zeros((part.shape[0], T - part.shape[1]), part.dtype)], axis=1)
                at = at[:-1] + (slice(None),)
                pltpu.store(self.ref.at[at], part, mask=_iota(part.shape, 1) >= 0)

    def __getitem__(self, idx):
        return jnp.concatenate([self.ref[at] for at in self.panels(idx)], axis=1)


def _buffers():
    buf = lambda shape, dtype, n=None: [buf(shape, dtype)] * n if n else jax.ShapeDtypeStruct(shape, dtype)
    wbuf = lambda n, l: buf((n, 7 ** l, D // 2 >> l, 4 * T >> l), I32)
    xshape = lambda l: (7 ** l, D // 2 >> l, C >> l)
    return [buf((NC, D, C), F32), buf((4, 3 * D // 2, 2 * T), I32),
            wbuf(3, LEV["aqkv"]), wbuf(1, LEV["ao"]), wbuf(3, LEV["bqkv"]), wbuf(1, LEV["bo"]),
            buf((NC,) + xshape(LEV["aqkv"]), I32), buf(xshape(LEV["ao"]), I32, 2), buf(xshape(LEV["bqkv"]), I32, 2),
            buf(xshape(LEV["bo"]), I32, 2), buf((D, C), F32, 6), buf((NP, PR, C), I32), buf((NC, NP, PR, C), I32),
            buf((NP, 64, 4 * DH), F32), buf((NP, 64, 4 * DH), BF16),
            buf((NC, H, C // 2, T), I32), buf((NC, H, 32, C), BF16), buf((NC, H, 16, C), I32),
            buf((D, C), F32, 2), buf((NC, D, C), F32), buf((2 * T, T), F32, H),
            [buf((D // 4, C // 4), F32, 5), buf((D // 2, C // 2), F32, 5)], buf((T, T), F32), buf((4, D, 2 * T), F32)]


def _token(*vals):
    regs = []
    for v in vals:
        v = _i32(v)
        regs += [v[r:r + 8, l:l + T] for r in range(0, v.shape[0], 8) for l in range(0, v.shape[1], T)]
    return _chains(jnp.bitwise_or, regs)


def _after(w, tokens):
    if not tokens:
        return w
    strips = _rows8(w)
    for i, tok in enumerate(tokens):
        j = i * len(strips) // len(tokens)
        n = min(tok.shape[1], w.shape[1])
        head = jnp.where(_iota((8, n), 1) * _iota((8, n), 1) == 2, tok[:, :n], strips[j][:, :n])
        strips[j] = jnp.concatenate([head, strips[j][:, n:]], axis=1) if n < w.shape[1] else head
    del tokens[:]
    return jnp.concatenate(strips, axis=0)


def _strassen(w_ref, x_ref, tmp, level, base, sink, tokens):
    if level == 0:
        n = w_ref.ref.shape[-2]
        for lo in range(0, n, min(RS, n)):
            x = x_ref[base]
            x = jnp.concatenate([x, jnp.zeros((w_ref.cols // 2 - x.shape[0], x.shape[1]), I32)], axis=0)
            out = _dot(_bf16(_after(w_ref[base, lo:lo + min(RS, n), :], tokens)), _bf16(x))
            for r in range(0, out.shape[0], 16):
                sink(2 * lo + r, 0, out[r:r + 16])
            yield
        return
    m = tmp[level - 1]
    regs = {}
    inreg = INREG if level < len(tmp) else ()
    rows, cols = m[0].ref.shape[1], m[0].cols

    def step(keep, quad, add=(), sub=()):
        def put(r, c, v):
            at = (slice(r, r + 16), slice(c, c + v.shape[1]))
            if keep in inreg:
                regs[keep, r, c] = v
            elif keep is not None:
                m[keep][at] = v
            if quad is not None:
                for i in add:
                    v = v + (regs[i, r, c] if i in inreg else m[i][at])
                for i in sub:
                    v = v - (regs[i, r, c] if i in inreg else m[i][at])
                sink(quad[0] * rows + r, quad[1] * cols + c, v)
        return put

    steps = [step(0, None), step(1, (1, 0), (0,)), step(2, None), step(3, (0, 1), (2,)), step(4, None),
             step(None, (1, 1), (4, 2), (0,)), step(None, (0, 0), (4, 1), (3,))]
    for i, put in enumerate(steps):
        yield from _strassen(w_ref, x_ref, tmp, level - 1, base + i * 7 ** (level - 1), put, tokens)


def _seq(*tasks):
    def gen():
        for g, _ in tasks:
            yield from g
    return gen(), [c for _, costs in tasks for c in costs]


def _par(main, *others, lead=1.0):
    def gen():
        total = sum(main[1])
        done, pos = [0] * len(others), 0
        for cost in main[1]:
            pos += cost
            for i, (g, costs) in enumerate(others):
                while done[i] < len(costs) and sum(costs[:done[i]]) * total * lead < pos * sum(costs):
                    next(g)
                    done[i] += 1
            next(main[0])
            yield
        for g, _ in (main,) + others:
            assert next(g, "end") == "end"
    return gen(), main[1]


def _idle(cost):
    n = -(-cost // 50)
    return iter([None] * n), [cost / n] * n


def _run(task):
    for _ in task[0]:
        pass


def _steps(n, cost):
    return lambda f: lambda *a: (f(*a), [cost] * n)


def _kernel(x_hbm, awqkv_hbm, wphi_hbm, awo_hbm, bwqkv_hbm, bwo_hbm, o_hbm,
            xio, wqkv, wphi, awo, bwo, sems,
            bufs):
    bufs = jax.tree.map(lambda ref, b: _Buf(ref, b.shape[-1]), bufs, _buffers())
    xs, wt, wa, woa, wb, wob, xa, xoa, xb, xob, ys, phik, phiq, acc, kvs, krep, vt, qs, oa, ob, ss, tmp, tri, yf = bufs

    due = []
    awqkv, bwqkv = wqkv.at[0], wqkv.at[1]

    def chunk(c):
        return pl.ds(c * C if isinstance(c, int) else pl.multiple_of(c * C, C), C)

    cuts = ((3 * T, 7 * T), (0, 3 * T), (7 * T, 3 * D))
    srcs = [(wphi_hbm, wphi)] + [(awqkv_hbm.at[:, a:b], awqkv.at[:, a:b]) for a, b in cuts]
    srcs += [(bwqkv_hbm.at[:, a:b], bwqkv.at[:, a:b]) for a, b in cuts]
    srcs += [(awo_hbm, awo), (bwo_hbm, bwo)]
    loads = [pltpu.make_async_copy(a, b, sems.at[2 * NC + i]) for i, (a, b) in enumerate(srcs)]
    x_in = lambda c: pltpu.make_async_copy(x_hbm.at[:, chunk(c)], xio.at[c], sems.at[c])
    x_out = lambda c: pltpu.make_async_copy(xio.at[c], o_hbm.at[:, chunk(c)], sems.at[NC + c])

    def x_last(i):
        r, l = ((1, 0), (0, 1), (1, 1), (0, 0))[i]
        r, n = (pl.ds(r * D // 2, D // 2), C // 2) if len(QS) == 4 else (slice(None), C // len(QS))
        l = l * n if len(QS) == 4 else (len(QS) - 1 - i) * n
        return pltpu.make_async_copy(xio.at[NC - 1, r, pl.ds(l, n)], o_hbm.at[r, pl.ds((NC - 1) * C + l, n)], sems.at[9 + 2 * NC + i])

    def start(when):
        for cp, t in zip(loads[:4] + [x_in(0), x_in(1), x_in(2), loads[4], x_in(3)] + loads[5:], DM):
            if t == when:
                cp.start()

    start(0)

    def transpose(src, level, lo=0, cols=None, shift=None):
        kp, cols = D >> level, cols or src.shape[1]

        def gen():
            for c0 in range(lo, cols, T):
                c1 = min(c0 + T, cols)
                at = slice(c0, c1) if shift is None else pl.ds(pl.multiple_of(shift + c0, T), T)
                out = [_i32(_bf16(_pack(src[k * kp:(k + 1) * kp, at].astype(F32))).T) for k in range(1 << level)]
                for k, w in enumerate(out):
                    wt[k, c0 // 2:c1 // 2, 0:kp] = w
                due.append(_token(*[w[:8, 0:min(kp, T)] for w in out]))
                yield
        return gen(), [120] * pl.cdiv(cols - lo, T)

    def weights(dst, j, level, get=None):
        kp = D >> level
        get = get or (lambda k, r: _unpack(wt[k, pl.ds((D * j + r) // 2, 8), 0:kp]))

        def gen():
            for r in range(0, kp, 16):
                ks = [jnp.concatenate([get(k, m * kp + r) for m in range(1 << level)], axis=0) for k in range(1 << level)]
                out = [_pack(p) for p in _split_lhs(ks)]
                for i, p in enumerate(out):
                    dst[j, i, r // 2:r // 2 + 8, :] = p
                due.append(_token(*[p[:, 0:min(kp, T)] for p in out]))
                yield
        return gen(), [60 * level ** 2] * (kp // 16)

    def stage(dst, level, get, tok=0):
        kp = D >> level

        def gen():
            for r in range(0, kp, 16):
                out = _split_rhs([get(k * kp + r) for k in range(1 << level)])
                for i, p in enumerate(out):
                    dst[i, r // 2:r // 2 + 8, :] = p
                due.append(_token(*out[tok:]))
                yield
        return gen(), [60 * level ** 2] * (kp // 16)

    def norm(c, dst, level, first=False):
        mean, rstd = [None] * (C // T), [None] * (C // T)

        def gen():
            for t in (2, 3, 0, 1):
                ls = slice(t * T, (t + 1) * T)
                for r in range(0, D, 2 * PR):
                    if first:
                        x = xio[c, r:r + 2 * PR, ls].astype(F32)
                        xs.at(c)[r:r + 2 * PR, ls] = x
                        rows = _rows8(x)
                    else:
                        rows = [xs.at(c).ref[t, pl.ds(r + o + i, 8, stride=7), :] for o in (0, PR) for i in range(7)]
                    if r == 0:
                        pivot, s1, s2 = _allreduce8(jnp.add, rows[0], (4, 2, 1)) * 0.125, [], []
                    rows = [v - pivot for v in rows]
                    s1 = [_chains(jnp.add, s1 + rows)]
                    s2 = [_chains(jnp.add, s2 + [v * v for v in rows])]
                    if r + 2 * PR == D:
                        m1, m2 = [_allreduce8(jnp.add, v[0], (4, 2, 1)) * (1.0 / D) for v in (s1, s2)]
                        mean[t] = jnp.concatenate([pivot + m1] * 2, axis=0)
                        rstd[t] = jnp.concatenate([lax.rsqrt(jnp.maximum(m2 - m1 * m1, 0.0) + 1e-5)] * 2, axis=0)
                    due.append(_token(s1[0], s2[0]))
                    yield
        get = lambda r: (xs.at(c)[r:r + 16, :] - jnp.concatenate(mean, axis=1)) * jnp.concatenate(rstd, axis=1)
        return _seq((gen(), [65] * (4 * C // T)), stage(dst, level, get, 4 * first))

    def matmul(w_ref, x_ref, level, sink):
        def gen():
            put = lambda r, c, v: sink(slice(r, r + 16), slice(c, c + v.shape[1]), v)
            for i, _ in enumerate(_strassen(w_ref, x_ref, tmp[2 - level:], level, 0, put, due)):
                if level < 2 or (i % YS == 0 and i):
                    yield
        return gen(), [2 * RS] * (7 * 112 // RS) if level == 1 else [28 * YS] * (48 // YS)

    def project(w_ref, j, x_ref, level, slot):
        def sink(r, l, v):
            ys[slot][r, l] = v
        return matmul(w_ref.at(j), x_ref, level, sink)

    low = _iota((8, C), 0) < 4
    a_norm = lambda c: norm(c, xa.at(c), LEV["aqkv"], True)
    a_proj = lambda j, c: project(wa, j, xa.at(c), LEV["aqkv"], j)

    @_steps(NP * C // T, 82)
    def a_features(j, c):
        for qi, qj in ((1, 0), (0, 1), (1, 1), (0, 0)):
            for p, t in [(4 * qi + p, 2 * qj + t) for p in range(4) for t in range(2)]:
                ls = slice(t * T, (t + 1) * T)
                phi = _hedgehog(ys[j][PR * p:PR * (p + 1), ls])
                dst = phiq.at(c) if j == 0 else phik
                dst[p, :, ls] = phi
                due.append(_token(phi))
                yield

    @_steps(2, 256)
    def a_state(final):
        rr = _iota((64, 4 * DH), 0)
        second = ((rr >= DH) & (rr < PR)) | (rr >= PR + 4)
        keep = second.astype(I32) == ((_iota((64, 4 * DH), 1) >> 1) & 1)
        for p in (4, 5, 6, 7, 0, 1, 2, 3):
            v1 = jnp.concatenate([ys[2][PR * p:PR * (p + 1), :], jnp.ones((8, C), F32)], axis=0).astype(BF16)
            part = _dot_nt(v1, _bf16(phik[p]))
            part = acc[p] + part
            if final:
                kvs[p] = jnp.where(keep, part, 0.0)
            else:
                acc[p] = part
            if p % 4 == 3:
                yield

    @_steps(2, 256)
    def a_read(c, i=0):
        for p in range(NP):
            nd = _dot(kvs[p], _bf16(_after(phiq.at(c)[p], due)))
            inv = _recip(nd[PR:] + 1e-6)
            sw = pltpu.roll(inv, 4, 0)
            i0, i1 = jnp.where(low, inv, sw), jnp.where(low, sw, inv)
            o = [a * b for a, b in zip(_rows8(nd[:PR]), [i0] * 3 + [inv] + [i1] * 3)]
            oa[i][PR * p:PR * (p + 1), :] = jnp.concatenate(o, axis=0)
            if p % 4 == 3:
                yield

    def residual(c, last=False):
        def sink(r, l, v):
            if last:
                xio[c, r, l] = (xs.at(c)[r, l] + v).astype(BF16)
            else:
                xs.at(c)[r, l] = xs.at(c)[r, l] + v
        return sink

    a_stage = lambda i=0: stage(xoa[i], LEV["ao"], lambda r: oa[i][r:r + 16, :])
    a_out = lambda c, i=0: matmul(woa.at(0), xoa[i], LEV["ao"], residual(c))
    b_norm = lambda c, i=0: norm(c, xb[i], LEV["bqkv"])
    b_proj = lambda j, i=0: project(wb, j, xb[i], LEV["bqkv"], 3 + j)
    b_stage = lambda c, i=0: stage(xob[i], LEV["bo"], lambda r: ob.at(c)[r:r + 16, :])
    b_out = lambda c, i=0: matmul(wob.at(0), xob[i], LEV["bo"], residual(c, True))

    @_steps(H, 40)
    def b_heads(j, c):
        for h in reversed(range(H)):
            r0 = PR * (h // 2) + 24 * (h % 2)
            y = ys[3 + j][r0:r0 + 32, :]
            if j == 1:
                k = _i32(_bf16(jnp.concatenate([_pack(y)] * 4, axis=0)).T)
                krep[c, h] = k
                due.append(_token(*[k[r - 8:r] for r in range(64, C // 2 + 1, 64)]))
            else:
                w = _rows8(y * (LOG2E * DH ** -0.5) if j == 0 else y)
                if h % 2 == 0:
                    w[3] = jnp.where(low, w[3], j / 2)
                else:
                    w[0] = jnp.where(low, j / 2, w[0])
                w = jnp.concatenate(w, axis=0)
                if j == 0:
                    w = _pack(w)
                (qs if j == 0 else vt)[c, h] = w
                due.append(_token(w if j == 0 else w[24:32] if h % 2 == 0 else w[0:8]))
            yield

    grp = _iota((16, T), 1) >> 5
    rr, ll = _iota((32, T), 0), _iota((32, T), 1)
    later = [(rr + 32 * j > ll) & (ll >= 32 * j) for j in range(4)]
    causal = _iota((T, T), 0) <= _iota((T, T), 1)
    tri[:, :] = causal.astype(F32)
    tpc = C // T
    ktile = lambda c, i, h, r, n: krep[c + i // tpc, h, pl.ds(i % tpc * T // 2 + r, n), :]
    low1 = _iota((8, T), 0) < 4

    def scores(c, i, h, back, ns):
        q = _i32(qs[c, h, :, i % tpc * T:(i % tpc + 1) * T])
        qbd = jnp.concatenate([jnp.where(grp == j, q, 0) for j in range(4)], axis=0)
        new = [ktile(c, i, h, 16 * j, 16) for j in range(4)]
        if back == 2:
            old = [ktile(c, i - 2, h, 16 * j, 16) for j in range(4)]
            ext = jnp.where(grp < 2, jnp.where(grp == 0, old[0], old[1]), jnp.where(grp == 2, old[2], old[3]))
            new = [ext, new[0]] + [jnp.where(grp >= j, new[j], old[j]) for j in range(1, 4)]
        if back >= 1:
            new.append(ktile(c, i - 1, h, 0, T // 2))
        keys = _after(jnp.concatenate(new, axis=0), due)
        cut = [keys.shape[0] // 8 * n // ns * 8 for n in range(ns + 1)]
        s = jnp.concatenate([_dot(_bf16(keys[a:b]), _bf16(qbd)) for a, b in zip(cut, cut[1:])], axis=0)
        if back == 2:
            rows = []
            for j in range(4):
                rows += _rows8(jnp.where(later[j], s[0:32], s[32 + 32 * j:64 + 32 * j]))
            rows += _rows8(s[32 + T:])
        else:
            rows = _rows8(jnp.where(causal, s[0:T], -1e9 * LOG2E)) + (_rows8(s[T:]) if back else [])
        mx = _allreduce8(jnp.maximum, _chains(jnp.maximum, rows), (4, 2, 1))
        ss[h][0:8 * len(rows), :] = jnp.concatenate(rows, axis=0)
        return mx

    def attend(c, i, h, back, mx):
        e = jnp.concatenate([jnp.exp2(v - mx) for v in _rows8(ss[h][0:min(back + 1, 2) * T, :])], axis=0)
        if back == 2:
            cur = e[0:T] * tri[:, :]
            e = jnp.concatenate([e[0:T] - cur, e[T:], cur], axis=0)
        elif back == 1:
            e = jnp.concatenate([e[T:], e[0:T]], axis=0)
        v = [vt[c + k // tpc, h, :, k % tpc * T:(k % tpc + 1) * T] for k in range(i - back, i + 1)]
        return _rows8(_dot(jnp.concatenate(v, axis=1), e.astype(BF16)))

    @_steps(2 * (C // T) * H // G, 48 * G)
    def b_attend(c, ns, LAG, first=False):
        items = [(i, h, min(i, 2) if first else 2) for i in range(C // T) for h in range(H)]
        groups = [items[n:n + G] for n in range(0, len(items), G)]
        pend, done = {}, {}
        for n in range(len(groups) + LAG):
            if n < len(groups) and not PVF:
                for it in groups[n]:
                    pend[it] = scores(c, *it, ns)
                yield
            if n >= LAG:
                for (i, h, back) in groups[n - LAG]:
                    done[h] = attend(c, i, h, back, pend.pop((i, h, back)))
                    if h % 2:
                        a, b = done[h - 1], done[h]
                        inv = _recip(jnp.where(low1, b[0], a[3]))
                        sw = pltpu.roll(inv, 4, 0)
                        i0, i1 = jnp.where(low1, sw, inv), jnp.where(low1, inv, sw)
                        o = [v * i0 for v in a[:3]] + [jnp.where(low1, a[3], b[0]) * sw] + [v * i1 for v in b[1:]]
                        ob[c, PR * (h // 2):PR * (h // 2 + 1), i * T:(i + 1) * T] = jnp.concatenate(o, axis=0)
                yield
            if n < len(groups) and PVF:
                for it in groups[n]:
                    pend[it] = scores(c, *it, ns)
                yield

    row = lambda n: (n & ~15) + ((n & 7) << 1) + ((n >> 3) & 1)
    m = row(_iota((4 * DH, DH), 0))
    sel = (((m - jnp.where(m >= PR, PR, 0)) >> 1) == _iota((4 * DH, DH), 1)).astype(F32).astype(BF16)
    r = _iota((D, 4 * DH), 0)
    perm = (((r & 3) * DH + (r >> 4)) == _iota((D, 4 * DH), 1)).astype(F32).astype(BF16)
    m = row(_iota((4 * DH, D), 0))
    head = jnp.where(m >= PR, 2, 0) + (m & 1)
    loads[0].wait()
    start(1)
    t = _dot_nt(sel, wphi[...])
    fold = [_dot(jnp.where((_iota((4 * DH, D), 1) & 15) == head + 4 * g, t, 0.0).astype(BF16), perm).astype(BF16)
            for g in range(4)]
    la = LEV["aqkv"]

    def folded(j):
        kp = D >> la

        def gen():
            for g in range(4):
                for k in range(1 << la):
                    yf[k, 4 * DH * g:4 * DH * (g + 1), 0:kp] = _dot(fold[g], _bf16(wt[k, pl.ds(D * j // 2 + PR * g, PR), 0:kp])) * LOG2E
                yield
        return _seq((gen(), [150] * 4), weights(wa, j, la, lambda k, r: yf[k, r:r + 16, 0:kp]))

    start(2)
    loads[1].wait()
    start(3)
    _run(_seq(transpose(awqkv, la, *cuts[0]), folded(1)))
    x_in(0).wait()
    start(4)
    _run(a_norm(0))
    loads[2].wait()
    loads[3].wait()
    start(5)
    del due[:]
    _run(_par(a_proj(1, 0), _seq(transpose(awqkv, la, *cuts[1]), folded(0), transpose(awqkv, la, *cuts[2]), weights(wa, 2, la))))
    lb = LEV["bqkv"]

    def section(task):
        del due[:]
        _run(task)

    def layer_pair(n, _):
        for p in range(NP):
            acc[p] = jnp.zeros((64, 4 * DH), F32)

        def features(c, _):
            pl.when(n == 0)(lambda: x_in(c + 1).wait())
            for j in (1, 2):
                pl.when((n == 0) & (c == j))(loads[3 + j].wait)
            skip = pl.multiple_of((c & 1) * 32, 32)
            more = weights(wb, 2 - c, lb, lambda k, r: _unpack(wt[k, pl.ds(skip + r // 2, 8), 0:D >> lb]))
            section(_par(_seq(a_proj(0, c), a_proj(2, c), a_state(False), a_proj(1, c + 1)),
                         _seq(_idle(Q['f0']), a_features(1, c), a_norm(c + 1), a_features(0, c),
                              transpose(wqkv.at[(c + 1) >> 1], lb, 0, 4 * T, (2 - c) * D - 2 * skip), more, _idle(Q['f1']))))

        lax.fori_loop(0, NC - 1, features, None)

        @pl.when(n == 0)
        def _():
            for cp in loads[6:]:
                cp.wait()

        lo = LEV["ao"]
        section(_seq(_par(a_proj(2, 3), a_features(1, 3)),
                     _par(_par(a_proj(0, 3), _seq(_idle(Q['m0']), a_state(True), _idle(Q['m1']), a_read(0), _par(_seq(a_read(1, 1), _idle(Q['m2'])), a_stage()))),
                          _seq(transpose(awo, lo), weights(woa, 0, lo))),
                     _par(a_out(0), _seq(a_stage(1), transpose(bwqkv, lb, *cuts[2]), weights(wb, 2, lb))),
                     _par(a_out(1, 1), b_norm(0), lead=Q['m4']),
                     _par(_seq(b_proj(1), b_proj(0), b_proj(2)),
                          _seq(b_norm(1, 1), a_features(0, 3), b_heads(1, 0), _idle(Q['m5'])))))
        section(_seq(_par(b_proj(1, 1), _seq(b_heads(0, 0), b_heads(2, 0))),
                     _par(_seq(_par(b_proj(0, 1), b_heads(1, 1)), _par(b_proj(2, 1), b_heads(0, 1)),
                               _par(_idle(Q['m3']), b_heads(2, 1))), b_attend(0, Q['ns0'], Q['lag0'], True),
                          _seq(transpose(bwo, LEV["bo"]), weights(wob, 0, LEV["bo"]), _idle(Q['m6'])))))

        def window(c, _):
            bs = [_seq()] * Q['bs'] + [b_stage(c - 1)]
            section(_par(_seq(a_read(c + 1), _par(_idle(Q['w1']), a_stage()), _par(a_out(c + 1), _seq(*bs[0:1])), _par(_idle(Q['w2']), b_norm(c + 1), lead=Q['w3']),
                              _par(b_proj(1), _seq(*bs[1:])), _par(b_proj(2), b_heads(1, c + 1)),
                              _par(b_proj(0), b_heads(2, c + 1)), _par(b_out(c - 1), b_heads(0, c + 1))),
                         _seq(_idle(Q['w0']), b_attend(c, Q['ns1'], Q['lag1'])), lead=Q['wl']))
            pl.when(n == 1)(lambda: x_out(c - 1).start())

        lax.fori_loop(1, NC - 1, window, None)
        section(_par(_seq(_par(_idle(Q['t0']), _seq(b_stage(2), a_norm(0))), b_out(2)),
                     _seq(b_attend(3, Q['ns3'], Q['lag3']), b_stage(3, 1), _idle(Q['t1']))))
        pl.when(n == 1)(lambda: x_out(2).start())
        steps = b_out(3, 1)[0]
        del due[:]
        for i in range(7):
            next(steps)
            if i in QS:
                pl.when(n == 1)(lambda: x_last(QS.index(i)).start())
        pl.when(n == 0)(lambda: section(a_proj(1, 0)))

    lax.fori_loop(0, 2, layer_pair, None)
    for c in range(NC - 1):
        x_out(c).wait()
    for i in range(len(QS)):
        x_last(i).wait()


@jax.jit
def pallas_interleave_layers__linear_kernel_hedgehog__sliding_block__prompt_kernel(
        A_x, A_wqkv, A_w_phi, A_wo, B_x, B_wqkv, B_wo):
    del B_x
    panels = lambda b: pltpu.VMEM(b.shape[:-2] + (pl.cdiv(b.shape[-1], T), b.shape[-2], T), b.dtype)
    out = pl.pallas_call(
        _kernel,
        out_shape=jax.ShapeDtypeStruct((D, S), BF16),
        in_specs=[pl.BlockSpec(memory_space=pl.ANY)] * 6,
        out_specs=pl.BlockSpec(memory_space=pl.ANY),
        scratch_shapes=[
            pltpu.VMEM((NC, D, C), BF16), pltpu.VMEM((2, D, 3 * D), BF16), pltpu.VMEM((D, DH), BF16),
            pltpu.VMEM((D, D), BF16), pltpu.VMEM((D, D), BF16),
            pltpu.SemaphoreType.DMA((13 + 2 * NC,)),
            jax.tree.map(panels, _buffers()),
        ],
        compiler_params=pltpu.CompilerParams(vmem_limit_bytes=100 << 20, flags=FLAGS or None),
    )(A_x.reshape(S, D).T, A_wqkv, A_w_phi.transpose(1, 0, 2).reshape(DH * H, DH), A_wo, B_wqkv, B_wo)
    return out.T.reshape(1, S, D)
```

```python
import jax
import jax.numpy as jnp
from jax import lax
import jax.experimental.pallas as pl
import jax.experimental.pallas.tpu as pltpu

S, D, H, DH = 2048, 448, 16, 28
NP = H // 2
PR = 2 * DH
T = 128
LOG2E = 1.4426950408889634
F32, BF16, I32 = jnp.float32, jnp.bfloat16, jnp.int32
C = 512
NC = S // C
LEV = dict(aqkv=1, ao=1, bqkv=2, bo=2)
Q = dict(s0=500, mq=3, p0=0, p1=4, p2=0, tok2=5, f0=400, f1=200, m0=300, m1=200, m2=50, m3=500, m7=0.85, m4=0.7, m5=800, m6=1000, ns0=4, lag0=4,
         w0=1, w1=1600, w2=6800, w3=1.0, wl=0.96, bs=1, ns1=4, lag1=3, t0=3200, t1=1, ns3=3, lag3=5)


def _iota(shape, axis):
    return lax.broadcasted_iota(I32, shape, axis)


def _dot(a, b):
    return jnp.dot(a, b, preferred_element_type=F32)


def _dot_nt(a, b):
    return lax.dot_general(a, b, (((1,), (1,)), ((), ())), preferred_element_type=F32)


def _tree(op, xs):
    xs = list(xs)
    while len(xs) > 1:
        xs = [op(xs[i], xs[i + 1]) if i + 1 < len(xs) else xs[i] for i in range(0, len(xs), 2)]
    return xs[0]


def _chains(op, xs, n=2):
    accs = list(xs[:n])
    for i, v in enumerate(xs[n:]):
        accs[i % n] = op(accs[i % n], v)
    return _tree(op, accs)


def _i32(x):
    return pltpu.bitcast(x, I32)


def _bf16(x):
    return pltpu.bitcast(x, BF16)


def _pack(x, exact=False):
    x = _i32(x) if exact else _i32(x) + 0x8000
    return jnp.concatenate([lax.shift_right_logical(x[r:r + 8], 16) | (x[r + 8:r + 16] & -65536)
                            for r in range(0, x.shape[0], 16)], axis=0)


def _unpack(w):
    return pltpu.bitcast(jnp.concatenate([w << 16, w & -65536], axis=0), F32)


def _rows8(x):
    return [x[r:r + 8] for r in range(0, x.shape[0], 8)]


def _allreduce8(op, v, shifts):
    for s in shifts:
        v = op(v, pltpu.roll(v, s, 0))
    return v


def _hedgehog(p):
    rows = _rows8(p)
    hi = _allreduce8(jnp.maximum, _tree(jnp.maximum, rows), (4, 2))
    lo = _allreduce8(jnp.minimum, _tree(jnp.minimum, rows), (4, 2))
    out = []
    for e in ([jnp.exp2(r - hi) for r in rows], [jnp.exp2(lo - r) for r in rows]):
        inv = _recip(_allreduce8(jnp.add, _tree(jnp.add, e), (4, 2)))
        out += [v * inv for v in e]
    return jnp.concatenate(out, axis=0)


def _add(u, v):
    return [x + y for x, y in zip(u, v)]


def _sub(u, v):
    return [x - y for x, y in zip(u, v)]


def _recip(x):
    r = pl.reciprocal(x, approx=True)
    return r * (2.0 - x * r)


def _split_lhs(ks):
    if len(ks) == 1:
        return [ks[0]]
    m, h = ks[0].shape[0] // 2, len(ks) // 2
    a11, a12 = [k[:m] for k in ks[:h]], [k[:m] for k in ks[h:]]
    a21, a22 = [k[m:] for k in ks[:h]], [k[m:] for k in ks[h:]]
    ops = [_add(a21, a22), a22, a11, _add(a11, a12), _add(a11, a22), _sub(a21, a11), _sub(a12, a22)]
    return [p for o in ops for p in _split_lhs(o)]


def _split_rhs(ks):
    if len(ks) == 1:
        return [_pack(ks[0])]
    n, h = ks[0].shape[1] // 2, len(ks) // 2
    b11, b12 = [k[:, :n] for k in ks[:h]], [k[:, n:] for k in ks[:h]]
    b21, b22 = [k[:, :n] for k in ks[h:]], [k[:, n:] for k in ks[h:]]
    ops = [b11, _sub(b21, b11), _sub(b12, b22), b22, _add(b11, b22), _add(b11, b12), _add(b21, b22)]
    return [p for o in ops for p in _split_rhs(o)]


class _Buf:
    def __init__(self, ref, cols):
        self.ref, self.cols = ref, cols

    def at(self, i):
        return _Buf(self.ref.at[i], self.cols)

    def panels(self, idx):
        idx = idx if isinstance(idx, tuple) else (idx,)
        idx += (slice(None),) * (len(self.ref.shape) - 1 - len(idx))
        lo, hi, _ = idx[-1].indices(self.cols)
        return [idx[:-2] + (l // T, idx[-2], slice(0, min(T, hi - l))) for l in range(lo, hi, T)]

    def __setitem__(self, idx, v):
        for i, at in enumerate(self.panels(idx)):
            part = v[:, i * T:(i + 1) * T]
            if self.ref.dtype == BF16:
                self.ref[at] = part.astype(BF16)
            else:
                if part.shape[1] < T:
                    part = jnp.concatenate([part, jnp.zeros((part.shape[0], T - part.shape[1]), part.dtype)], axis=1)
                at = at[:-1] + (slice(None),)
                pltpu.store(self.ref.at[at], part, mask=_iota(part.shape, 1) >= 0)

    def __getitem__(self, idx):
        return jnp.concatenate([self.ref[at] for at in self.panels(idx)], axis=1)


def _buffers():
    buf = lambda shape, dtype, n=None: [buf(shape, dtype)] * n if n else jax.ShapeDtypeStruct(shape, dtype)
    wbuf = lambda n, l: buf((n, 7 ** l, D // 2 >> l, 4 * T >> l), I32)
    xshape = lambda l: (7 ** l, D // 2 >> l, C >> l)
    return [buf((NC, D, C), F32), buf((4, 3 * D // 2, 2 * T), I32),
            wbuf(3, LEV["aqkv"]), wbuf(1, LEV["ao"]), wbuf(3, LEV["bqkv"]), wbuf(1, LEV["bo"]),
            buf((NC,) + xshape(LEV["aqkv"]), I32), buf(xshape(LEV["ao"]), I32, 2), buf(xshape(LEV["bqkv"]), I32, 2),
            buf(xshape(LEV["bo"]), I32, 2), buf((D, C), F32, 3), buf((NP, 2 * PR, C), BF16), buf((NC, NP, 2 * PR, C), BF16),
            buf((NP, 64, 4 * DH), F32), buf((NP, 64, 4 * DH), BF16),
            buf((NC, H, C // 2, T), I32), buf((NC, H, 32, C), BF16), buf((NC, H, 32, C), BF16),
            buf((D, C), F32, 2), buf((NC, D, C), F32), buf((2 * T, T), F32, H),
            [buf((D // 2, C // 2), F32, 5)] * 2, buf((T, T), F32), buf((4, D, 2 * T), F32)]


def _token(*vals):
    regs = []
    for v in vals:
        v = _i32(v)
        regs += [v[r:r + 8, l:l + T] for r in range(0, v.shape[0], 8) for l in range(0, v.shape[1], T)]
    return _chains(jnp.bitwise_or, regs)


def _after(w, tokens):
    if not tokens:
        return w
    strips = _rows8(w)
    for i, tok in enumerate(tokens):
        j = i * len(strips) // len(tokens)
        n = min(tok.shape[1], w.shape[1])
        head = jnp.where(_iota((8, n), 1) * _iota((8, n), 1) == 2, tok[:, :n], strips[j][:, :n])
        strips[j] = jnp.concatenate([head, strips[j][:, n:]], axis=1) if n < w.shape[1] else head
    del tokens[:]
    return jnp.concatenate(strips, axis=0)


def _strassen(w_ref, x_ref, m, level, base, sink, tokens):
    if level == 0:
        x = x_ref[base]
        x = jnp.concatenate([x, jnp.zeros((w_ref.cols // 2 - x.shape[0], x.shape[1]), I32)], axis=0)
        out = _dot(_bf16(_after(w_ref[base], tokens)), _bf16(x))
        for r in range(0, out.shape[0], 16):
            sink(r, 0, out[r:r + 16])
        yield
        return
    rows, cols = D // 2, C // 2
    if m is None:
        rows, cols, p = D // 4, C // 4, {}
        for i in range(7):
            next(_strassen(w_ref, x_ref, None, 0, base + i, lambda r, c, v: p.__setitem__((i, r), v), tokens))
            for r in range(0, rows, 16):
                if i == 3:
                    p[7, r], p[8, r] = p[2, r] - p[0, r], p[1, r] - p[3, r]
                    sink(rows + r, 0, p[0, r] + p[1, r])
                    sink(r, cols, p[2, r] + p[3, r])
                if i == 6:
                    sink(rows + r, cols, p[7, r] + p[4, r] + p[5, r])
                    sink(r, 0, p[8, r] + p[4, r] + p[6, r])
            if i in (3, 6):
                yield
        return

    def step(keep, quad, add=(), sub=()):
        def put(r, c, v):
            at = (slice(r, r + 16), slice(c, c + v.shape[1]))
            if keep is not None:
                m[keep][at] = v
            if quad is not None:
                for i in add:
                    v = v + m[i][at]
                for i in sub:
                    v = v - m[i][at]
                sink(quad[0] * rows + r, quad[1] * cols + c, v)
        return put

    steps = [step(0, None), step(1, (1, 0), (0,)), step(2, None), step(3, (0, 1), (2,)), step(4, None),
             step(None, (1, 1), (4, 2), (0,)), step(None, (0, 0), (4, 1), (3,))]
    for i, put in enumerate(steps):
        yield from _strassen(w_ref, x_ref, None, level - 1, base + i * 7 ** (level - 1), put, tokens)


def _seq(*tasks):
    def gen():
        for g, _ in tasks:
            yield from g
    return gen(), [c for _, costs in tasks for c in costs]


def _par(main, *others, lead=1.0):
    def gen():
        total = sum(main[1])
        done, pos = [0] * len(others), 0
        for cost in main[1]:
            pos += cost
            for i, (g, costs) in enumerate(others):
                while done[i] < len(costs) and sum(costs[:done[i]]) * total * lead < pos * sum(costs):
                    next(g)
                    done[i] += 1
            next(main[0])
            yield
        for g, _ in (main,) + others:
            assert next(g, "end") == "end"
    return gen(), main[1]


def _idle(cost):
    n = -(-cost // 50)
    return iter([None] * n), [cost / n] * n


def _cut(task, n):
    return (next(task[0]) for _ in range(n)), task[1][:n]


def _run(task):
    for _ in task[0]:
        pass


def _steps(n, cost):
    return lambda f: lambda *a: (f(*a), [cost] * n)


def _kernel(x_hbm, awqkv_hbm, wphi_hbm, awo_hbm, bwqkv_hbm, bwo_hbm, o_hbm,
            xio, wqkv, wphi, awo, bwo, sems,
            bufs):
    bufs = jax.tree.map(lambda ref, b: _Buf(ref, b.shape[-1]), bufs, _buffers())
    xs, wt, wa, woa, wb, wob, xa, xoa, xb, xob, ys, phik, phiq, acc, kvs, krep, vt, qs, oa, ob, ss, tmp, tri, yf = bufs

    due = []
    awqkv, bwqkv = wqkv.at[0], wqkv.at[1]

    def chunk(c):
        return pl.ds(c * C if isinstance(c, int) else pl.multiple_of(c * C, C), C)

    cuts = ((3 * T, 7 * T), (0, 3 * T), (7 * T, 3 * D))
    srcs = [(wphi_hbm, wphi)] + [(awqkv_hbm.at[:, a:b], awqkv.at[:, a:b]) for a, b in cuts]
    srcs += [(bwqkv_hbm.at[:, a:b], bwqkv.at[:, a:b]) for a, b in cuts]
    srcs += [(awo_hbm, awo), (bwo_hbm, bwo)]
    loads = [pltpu.make_async_copy(a, b, sems.at[2 * NC + i]) for i, (a, b) in enumerate(srcs)]
    x_in = lambda c: pltpu.make_async_copy(x_hbm.at[:, chunk(c)], xio.at[c], sems.at[c])
    x_out = lambda c: pltpu.make_async_copy(xio.at[c], o_hbm.at[:, chunk(c)], sems.at[NC + c])

    def x_last(i):
        r, l = ((1, 0), (0, 1), (1, 1), (0, 0))[i]
        r, l = pl.ds(r * D // 2, D // 2), l * C // 2
        return pltpu.make_async_copy(xio.at[NC - 1, r, pl.ds(l, C // 2)], o_hbm.at[r, pl.ds((NC - 1) * C + l, C // 2)],
                                     sems.at[9 + 2 * NC + i])

    for cp in (loads[0], loads[1], x_in(0)):
        cp.start()

    def transpose(src, level, lo=0, cols=None, shift=None):
        kp, cols = D >> level, cols or src.shape[1]

        def gen():
            for c0 in range(lo, cols, T):
                c1 = min(c0 + T, cols)
                at = slice(c0, c1) if shift is None else pl.ds(pl.multiple_of(shift + c0, T), T)
                out = [_i32(_bf16(_pack(src[k * kp:(k + 1) * kp, at].astype(F32), True)).T) for k in range(1 << level)]
                for k, w in enumerate(out):
                    wt[k, c0 // 2:c1 // 2, 0:kp] = w
                due.append(_token(*[w[:8, 0:min(kp, T)] for w in out]))
                yield
        return gen(), [120] * pl.cdiv(cols - lo, T)

    def weights(dst, j, level, get=None):
        kp = D >> level
        get = get or (lambda k, r: _unpack(wt[k, pl.ds((D * j + r) // 2, 8), 0:kp]))

        def gen():
            for r in range(0, kp, 16):
                ks = [jnp.concatenate([get(k, m * kp + r) for m in range(1 << level)], axis=0) for k in range(1 << level)]
                out = [_pack(p) for p in _split_lhs(ks)]
                for i, p in enumerate(out):
                    dst[j, i, r // 2:r // 2 + 8, :] = p
                    if i % 7 == 6:
                        due.append(_token(*[p[:, 0:min(kp, T)] for p in out[i - 2:i + 1]]))
                        yield
        return gen(), [60 if level == 1 else 28] * (kp // 16 * 7 ** (level - 1))

    def stage(dst, level, get, tok=0):
        kp = D >> level

        def gen():
            for r in range(0, kp, 16):
                out = _split_rhs([get(k * kp + r) for k in range(1 << level)])
                for i, p in enumerate(out):
                    dst[i, r // 2:r // 2 + 8, :] = p
                    if i % 7 == 6:
                        due.append(_token(*out[i - 6 + (tok if level == 1 else Q['tok2']):i + 1]))
                        yield
        return gen(), [60 if level == 1 else 32] * (kp // 16 * 7 ** (level - 1))

    def norm(c, dst, level, first=False):
        mean, rstd = [None] * (C // T), [None] * (C // T)

        def gen():
            for t in (2, 3, 0, 1):
                ls = slice(t * T, (t + 1) * T)
                for r in range(0, D, 2 * PR):
                    if first:
                        x = xio[c, r:r + 2 * PR, ls].astype(F32)
                        xs.at(c)[r:r + 2 * PR, ls] = x
                        rows = _rows8(x)
                    else:
                        rows = [xs.at(c).ref[t, pl.ds(r + o + i, 8, stride=7), :] for o in (0, PR) for i in range(7)]
                    if r == 0:
                        pivot, s1, s2 = _allreduce8(jnp.add, rows[0], (4, 2, 1)) * 0.125, [], []
                    rows = [v - pivot for v in rows]
                    s1 = [_chains(jnp.add, s1 + rows)]
                    s2 = [_chains(jnp.add, s2 + [v * v for v in rows])]
                    if r + 2 * PR == D:
                        m1, m2 = [_allreduce8(jnp.add, v[0], (4, 2, 1)) * (1.0 / D) for v in (s1, s2)]
                        mean[t] = jnp.concatenate([pivot + m1] * 2, axis=0)
                        rstd[t] = jnp.concatenate([lax.rsqrt(jnp.maximum(m2 - m1 * m1, 0.0) + 1e-5)] * 2, axis=0)
                    due.append(_token(s1[0], s2[0]))
                    yield
        get = lambda r: (xs.at(c)[r:r + 16, :] - jnp.concatenate(mean, axis=1)) * jnp.concatenate(rstd, axis=1)
        return _seq((gen(), [65] * (4 * C // T)), stage(dst, level, get, 4 * first))

    def matmul(w_ref, x_ref, level, sink, bank=0):
        put = lambda r, c, v: sink(slice(r, r + 16), slice(c, c + v.shape[1]), v)
        return _strassen(w_ref, x_ref, tmp[bank], level, 0, put, due), [224] * 7 if level == 1 else [112, 84] * 7

    def project(w_ref, j, x_ref, level, slot):
        def sink(r, l, v):
            ys[slot][r, l] = v
        return matmul(w_ref.at(j), x_ref, level, sink, int(slot == 0))

    low = _iota((8, C), 0) < 4
    a_norm = lambda c: norm(c, xa.at(c), LEV["aqkv"], True)
    a_proj = lambda j, c: project(wa, j, xa.at(c), LEV["aqkv"], j)

    @_steps(NP * C // T, 82)
    def a_features(j, c):
        for qi, qj in ((1, 0), (0, 1), (1, 1), (0, 0)):
            for p, t in [(4 * qi + p, 2 * qj + t) for p in range(4) for t in range(2)]:
                ls = slice(t * T, (t + 1) * T)
                phi = _hedgehog(ys[j][PR * p:PR * (p + 1), ls])
                dst = phiq.at(c) if j == 0 else phik
                dst[p, :, ls] = phi
                due.append(_token(*_rows8(phi)[1::2]))
                yield

    @_steps(2, 256)
    def a_state(final):
        rr = _iota((64, 4 * DH), 0)
        second = ((rr >= DH) & (rr < PR)) | (rr >= PR + 4)
        keep = second.astype(I32) == (_iota((64, 4 * DH), 1) & 1)
        for p in (4, 5, 6, 7, 0, 1, 2, 3):
            v1 = jnp.concatenate([ys[2][PR * p:PR * (p + 1), :], jnp.ones((8, C), F32)], axis=0).astype(BF16)
            part = _dot_nt(v1, phik[p])
            part = acc[p] + part
            if final:
                kvs[p] = jnp.where(keep, part, 0.0)
                acc[p] = jnp.zeros_like(part)
            else:
                acc[p] = part
            if p % 4 == 3:
                yield

    @_steps(2, 256)
    def a_read(c, i=0):
        for p in range(NP):
            nd = _dot(kvs[p], _bf16(_after(_i32(phiq.at(c)[p]), due)))
            inv = _recip(nd[PR:] + 1e-6)
            sw = pltpu.roll(inv, 4, 0)
            i0, i1 = jnp.where(low, inv, sw), jnp.where(low, sw, inv)
            o = [a * b for a, b in zip(_rows8(nd[:PR]), [i0] * 3 + [inv] + [i1] * 3)]
            oa[i][PR * p:PR * (p + 1), :] = jnp.concatenate(o, axis=0)
            if p % 4 == 3:
                yield

    def residual(c, last=False):
        def sink(r, l, v):
            if last:
                xio[c, r, l] = (xs.at(c)[r, l] + v).astype(BF16)
            else:
                xs.at(c)[r, l] = xs.at(c)[r, l] + v
        return sink

    a_stage = lambda i=0: stage(xoa[i], LEV["ao"], lambda r: oa[i][r:r + 16, :])
    a_out = lambda c, i=0: matmul(woa.at(0), xoa[i], LEV["ao"], residual(c))
    b_norm = lambda c, i=0: norm(c, xb[i], LEV["bqkv"])
    b_stage = lambda c, i=0: stage(xob[i], LEV["bo"], lambda r: ob.at(c)[r:r + 16, :])
    b_out = lambda c, i=0: matmul(wob.at(0), xob[i], LEV["bo"], residual(c, True))

    def b_proj(j, c, i=0):
        got = {}

        def sink(r, l, v):
            got[r.start, l.start], got[r.start + 8, l.start] = v[0:8], v[8:16]
            for h in range(H):
                r0 = PR * (h // 2) + 24 * (h % 2)
                if not r.start <= r0 + 24 < r.stop:
                    continue
                w = [got[r0 + o, l.start] for o in range(0, 32, 8)]
                if j == 1:
                    k = _i32(jnp.concatenate(w * 4, axis=0).astype(BF16).T)
                    krep[c, h, l.start // 2:l.stop // 2, :] = k
                    continue
                if j == 0:
                    w = [u * (LOG2E * DH ** -0.5) for u in w]
                if h % 2 == 0:
                    w[3] = jnp.where(low1, w[3], j / 2)
                else:
                    w[0] = jnp.where(low1, j / 2, w[0])
                w = jnp.concatenate(w, axis=0)
                (qs if j == 0 else vt)[c, h, :, l] = w
        return matmul(wb.at(j), xb[i], LEV["bqkv"], sink)

    grp = _iota((16, T), 1) >> 5
    rr, ll = _iota((32, T), 0), _iota((32, T), 1)
    later = [(rr + 32 * j > ll) & (ll >= 32 * j) for j in range(4)]
    causal = _iota((T, T), 0) <= _iota((T, T), 1)
    tri[:, :] = causal.astype(F32)
    tpc = C // T
    ktile = lambda c, i, h, r, n: krep[c + i // tpc, h, pl.ds(i % tpc * T // 2 + r, n), :]
    low1 = _iota((8, T), 0) < 4

    def scores(c, i, h, back, ns):
        q = _i32(qs[c, h, :, i % tpc * T:(i % tpc + 1) * T])
        qbd = jnp.concatenate([jnp.where(grp == j, q, 0) for j in range(4)], axis=0)
        new = [ktile(c, i, h, 16 * j, 16) for j in range(4)]
        if back == 2:
            old = [ktile(c, i - 2, h, 16 * j, 16) for j in range(4)]
            ext = jnp.where(grp < 2, jnp.where(grp == 0, old[0], old[1]), jnp.where(grp == 2, old[2], old[3]))
            new = [ext, new[0]] + [jnp.where(grp >= j, new[j], old[j]) for j in range(1, 4)]
        if back >= 1:
            new.append(ktile(c, i - 1, h, 0, T // 2))
        keys = _after(jnp.concatenate(new, axis=0), due)
        cut = [keys.shape[0] // 8 * n // ns * 8 for n in range(ns + 1)]
        s = jnp.concatenate([_dot(_bf16(keys[a:b]), _bf16(qbd)) for a, b in zip(cut, cut[1:])], axis=0)
        if back == 2:
            rows = []
            for j in range(4):
                rows += _rows8(jnp.where(later[j], s[0:32], s[32 + 32 * j:64 + 32 * j]))
            rows += _rows8(s[32 + T:])
        else:
            rows = _rows8(jnp.where(causal, s[0:T], -1e9 * LOG2E)) + (_rows8(s[T:]) if back else [])
        mx = _allreduce8(jnp.maximum, _chains(jnp.maximum, rows), (4, 2, 1))
        ss[h][0:8 * len(rows), :] = jnp.concatenate(rows, axis=0)
        return mx

    def attend(c, i, h, back, mx):
        e = jnp.concatenate([jnp.exp2(v - mx) for v in _rows8(ss[h][0:min(back + 1, 2) * T, :])], axis=0)
        if back == 2:
            cur = e[0:T] * tri[:, :]
            e = jnp.concatenate([e[0:T] - cur, e[T:], cur], axis=0)
        elif back == 1:
            e = jnp.concatenate([e[T:], e[0:T]], axis=0)
        v = [vt[c + k // tpc, h, :, k % tpc * T:(k % tpc + 1) * T] for k in range(i - back, i + 1)]
        return _rows8(_dot(jnp.concatenate(v, axis=1), e.astype(BF16)))

    @_steps(2 * tpc * H, 48)
    def b_attend(c, ns, lag, first=False):
        items = [(i, h, min(i, 2) if first else 2) for i in range(tpc) for h in range(H)]
        mx, done = {}, {}
        for n in range(len(items) + lag):
            if n < len(items):
                mx[n] = scores(c, *items[n], ns)
                yield
            if n >= lag:
                i, h, back = items[n - lag]
                done[h] = attend(c, i, h, back, mx.pop(n - lag))
                if h % 2:
                    a, b = done[h - 1], done[h]
                    inv = _recip(jnp.where(low1, b[0], a[3]))
                    sw = pltpu.roll(inv, 4, 0)
                    i0, i1 = jnp.where(low1, sw, inv), jnp.where(low1, inv, sw)
                    o = [v * i0 for v in a[:3]] + [jnp.where(low1, a[3], b[0]) * sw] + [v * i1 for v in b[1:]]
                    ob[c, PR * (h // 2):PR * (h // 2 + 1), i * T:(i + 1) * T] = jnp.concatenate(o, axis=0)
                yield

    row = lambda n: (n & ~15) + ((n & 7) << 1) + ((n >> 3) & 1)
    m = row(_iota((4 * DH, DH), 0))
    sel = (((m - jnp.where(m >= PR, PR, 0)) >> 1) == _iota((4 * DH, DH), 1)).astype(F32).astype(BF16)
    r = _iota((D, 4 * DH), 0)
    perm = (((r & 3) * DH + (r >> 4)) == _iota((D, 4 * DH), 1)).astype(F32).astype(BF16)
    m = row(_iota((4 * DH, D), 0))
    head = jnp.where(m >= PR, 2, 0) + (m & 1)
    for p in range(NP):
        acc[p] = jnp.zeros((64, 4 * DH), F32)
    loads[0].wait()
    t = _dot_nt(sel, wphi[...])
    fold = [_dot(jnp.where((_iota((4 * DH, D), 1) & 15) == head + 4 * g, t, 0.0).astype(BF16), perm).astype(BF16)
            for g in range(4)]
    la = LEV["aqkv"]

    def folded(j):
        kp = D >> la

        def gen():
            for g in range(4):
                for k in range(1 << la):
                    yf[k, 4 * DH * g:4 * DH * (g + 1), 0:kp] = _dot(fold[g], _bf16(wt[k, pl.ds(D * j // 2 + PR * g, PR), 0:kp])) * LOG2E
                yield
        return _seq((gen(), [150] * 4), weights(wa, j, la, lambda k, r: yf[k, r:r + 16, 0:kp]))

    loads[2].start()
    loads[3].start()
    loads[1].wait()
    _run(_seq(transpose(awqkv, la, *cuts[0]), folded(1)))
    x_in(0).wait()
    for cp in [x_in(1), x_in(2), loads[4], x_in(3)] + loads[5:]:
        cp.start()
    _run(a_norm(0))
    wait = lambda cp: ((cp.wait() for _ in range(1)), [1])
    del due[:]
    _run(_par(a_proj(1, 0), _seq(_idle(Q['s0']), wait(loads[2]), transpose(awqkv, la, *cuts[1]), folded(0),
                                 wait(loads[3]), transpose(awqkv, la, *cuts[2]), weights(wa, 2, la))))
    lb = LEV["bqkv"]

    def section(task):
        del due[:]
        _run(task)

    def layer_pair(n, _):

        def features(c, _):
            pl.when(n == 0)(lambda: x_in(c + 1).wait())
            for j in (1, 2):
                pl.when((n == 0) & (c == j))(loads[3 + j].wait)
            skip = pl.multiple_of((c & 1) * 32, 32)
            more = weights(wb, 2 - c, lb, lambda k, r: _unpack(wt[k, pl.ds(skip + r // 2, 8), 0:D >> lb]))
            section(_par(_seq(a_proj(0, c), a_proj(2, c), a_state(False), a_proj(1, c + 1)),
                         _seq(_idle(Q['f0']), a_features(1, c), a_norm(c + 1), a_features(0, c),
                              transpose(wqkv.at[(c + 1) >> 1], lb, 0, 4 * T, (c & 1) * 3 * T), more, _idle(Q['f1']))))

        lax.fori_loop(0, NC - 1, features, None)

        @pl.when(n == 0)
        def _():
            for cp in loads[6:]:
                cp.wait()

        lo = LEV["ao"]
        q3 = a_proj(0, 3)
        prep = [transpose(awo, lo), weights(woa, 0, lo), transpose(bwqkv, lb, *cuts[2]), weights(wb, 2, lb)]
        late = [a_features(0, 3)]
        section(_seq(_par(a_proj(2, 3), _seq(a_features(1, 3), *prep[:Q['p0']])),
                     _par(_par(_cut(q3, Q['mq']), _seq(_idle(Q['m0']), a_state(True), _idle(Q['m1']), a_read(0),
                                                       _par(_seq(a_read(1, 1), _idle(Q['m2'])), a_stage()))),
                          _seq(*prep[Q['p0']:2])),
                     _par(a_out(0), _seq(a_stage(1), *prep[2:Q['p1']])),
                     _par(_seq(a_out(1, 1), _cut(q3, 7 - Q['mq'])), b_norm(0), lead=Q['m4']),
                     _par(_seq(b_proj(1, 0), b_proj(0, 0), b_proj(2, 0)),
                          _seq(*prep[Q['p1']:], b_norm(1, 1), *late[:Q['p2']], _idle(Q['m5'])))))
        section(_par(_seq(*[b_proj(j, 1, 1) for j in (1, 0, 2)]),
                     _seq(_idle(Q['m3']), b_attend(0, Q['ns0'], Q['lag0'], True)),
                     _seq(*late[Q['p2']:], transpose(bwo, LEV["bo"]), weights(wob, 0, LEV["bo"]), _idle(Q['m6'])), lead=Q['m7']))

        def window(c, _):
            bs = [_seq()] * Q['bs'] + [b_stage(c - 1)]
            section(_par(_seq(a_read(c + 1), _par(_idle(Q['w1']), a_stage()), _par(a_out(c + 1), _seq(*bs[0:1])), _par(_idle(Q['w2']), b_norm(c + 1), lead=Q['w3']),
                              _par(_seq(*[b_proj(j, c + 1) for j in (1, 0, 2)]), _seq(*bs[1:])), b_out(c - 1)),
                         _seq(_idle(Q['w0']), b_attend(c, Q['ns1'], Q['lag1'])), lead=Q['wl']))
            pl.when(n == 1)(lambda: x_out(c - 1).start())

        lax.fori_loop(1, NC - 1, window, None)
        section(_par(_seq(_par(_idle(Q['t0']), _seq(b_stage(2), a_norm(0))), b_out(2)),
                     _seq(b_attend(3, Q['ns3'], Q['lag3']), b_stage(3, 1), _idle(Q['t1']))))
        pl.when(n == 1)(lambda: x_out(2).start())
        steps = b_out(3, 1)[0]
        del due[:]
        for i in range(7):
            for _ in range(LEV["bo"]):
                next(steps)
            if i in (1, 3, 5, 6):
                pl.when(n == 1)(lambda: x_last(i // 2).start())
        pl.when(n == 0)(lambda: section(a_proj(1, 0)))

    lax.fori_loop(0, 2, layer_pair, None)
    for c in range(NC - 1):
        x_out(c).wait()
    for i in range(4):
        x_last(i).wait()


@jax.jit
def pallas_interleave_layers__linear_kernel_hedgehog__sliding_block__prompt_kernel(
        A_x, A_wqkv, A_w_phi, A_wo, B_x, B_wqkv, B_wo):
    del B_x
    panels = lambda b: pltpu.VMEM(b.shape[:-2] + (pl.cdiv(b.shape[-1], T), b.shape[-2], T), b.dtype)
    out = pl.pallas_call(
        _kernel,
        out_shape=jax.ShapeDtypeStruct((D, S), BF16),
        in_specs=[pl.BlockSpec(memory_space=pl.ANY)] * 6,
        out_specs=pl.BlockSpec(memory_space=pl.ANY),
        scratch_shapes=[
            pltpu.VMEM((NC, D, C), BF16), pltpu.VMEM((2, D, 3 * D), BF16), pltpu.VMEM((D, DH), BF16),
            pltpu.VMEM((D, D), BF16), pltpu.VMEM((D, D), BF16),
            pltpu.SemaphoreType.DMA((13 + 2 * NC,)),
            jax.tree.map(panels, _buffers()),
        ],
        compiler_params=pltpu.CompilerParams(vmem_limit_bytes=100 << 20),
    )(A_x.reshape(S, D).T, A_wqkv, A_w_phi.transpose(1, 0, 2).reshape(DH * H, DH), A_wo, B_wqkv, B_wo)
    return out.T.reshape(1, S, D)
```
